```python
import jax
import jax.numpy as jnp

def _softmax(x, axis=-1):
    return jax.nn.softmax(x, axis=axis)
def _gelu(x):
    return jax.nn.gelu(x, approximate=True)
def _silu(x):
    return jax.nn.silu(x)
def _sigmoid(x):
    return jax.nn.sigmoid(x)
def _layernorm(x, axis=-1, eps=1e-5):
    m = jnp.mean(x, axis=axis, keepdims=True)
    v = jnp.var(x, axis=axis, keepdims=True)
    return (x - m) / jnp.sqrt(v + eps)
def _scatter_add(tgt, idx, src, axis=0):
    return tgt.at[idx].add(src)
def _segment_sum(src, seg, n):
    return jax.ops.segment_sum(src, seg, n)
class _Rng:
    def __init__(self, key):
        self._k = key
    def _next(self):
        self._k, sub = jax.random.split(self._k)
        return sub
    def normal(self, shape):
        return jax.random.normal(self._next(), shape, dtype=jnp.bfloat16)
    def randint(self, lo, hi, shape):
        return jax.random.randint(self._next(), shape, lo, hi, dtype=jnp.int32)
    def uniform(self, shape, lo=0.0, hi=1.0):
        return jax.random.uniform(self._next(), shape, jnp.bfloat16, lo, hi)
    def permutation(self, n):
        return jax.random.permutation(self._next(), n)


kernel_name = 'concat_heads__gqa_block_cached__gqa_block_cached__near_ridge'

def setup_inputs():
    _rng = _Rng(jax.random.key(int.from_bytes(__import__("os").urandom(4), "little")))
    _w = (lambda a: (lambda t: t.astype(jnp.bfloat16) if jnp.issubdtype(t.dtype, jnp.floating) else t)(jnp.asarray(a)))
    def _A_setup():
        B, Sq, D = 8, 256, 640
        Hq, Hkv, Sk, Dh = 32, 32, 1024, 192
        assert Hq % Hkv == 0, (Hq, Hkv)
        return {
            "x": _w((lambda *s: _rng.normal(s) * 0.05)(B, Sq, D)),
            "k_cache": _w((lambda *s: _rng.normal(s) * 0.05)(B, Hkv, Sk, Dh)),
            "v_cache": _w((lambda *s: _rng.normal(s) * 0.05)(B, Hkv, Sk, Dh)),
            "wq": _w((lambda *s: _rng.normal(s) * 0.05)(D, Hq * Dh) * (D ** -0.5)),
            "wo": _w((lambda *s: _rng.normal(s) * 0.05)(Hq * Dh, D) * ((Hq * Dh) ** -0.5)),
        }
    _A_in = _A_setup()

    def _B_setup():
        B, Sq, D = 8, 256, 640
        Hq, Hkv, Sk, Dh = 32, 32, 1024, 192
        assert Hq % Hkv == 0, (Hq, Hkv)
        return {
            "x": _w((lambda *s: _rng.normal(s) * 0.05)(B, Sq, D)),
            "k_cache": _w((lambda *s: _rng.normal(s) * 0.05)(B, Hkv, Sk, Dh)),
            "v_cache": _w((lambda *s: _rng.normal(s) * 0.05)(B, Hkv, Sk, Dh)),
            "wq": _w((lambda *s: _rng.normal(s) * 0.05)(D, Hq * Dh) * (D ** -0.5)),
            "wo": _w((lambda *s: _rng.normal(s) * 0.05)(Hq * Dh, D) * ((Hq * Dh) ** -0.5)),
        }
    _B_in = _B_setup()

    return {
        "A_x": _A_in["x"],
        "A_k_cache": _A_in["k_cache"],
        "A_v_cache": _A_in["v_cache"],
        "A_wq": _A_in["wq"],
        "A_wo": _A_in["wo"],
        "B_x": _B_in["x"],
        "B_k_cache": _B_in["k_cache"],
        "B_v_cache": _B_in["v_cache"],
        "B_wq": _B_in["wq"],
        "B_wo": _B_in["wo"],
    }

def reference(A_x, A_k_cache, A_v_cache, A_wq, A_wo, B_x, B_k_cache, B_v_cache, B_wq, B_wo):
    def _A_ref(x, k_cache, v_cache, wq, wo):
        B, Sq, D = x.shape
        Hq, Dh = 32, 192
        Hkv = k_cache.shape[1]
        rep = Hq // Hkv
        q = (lambda x, *d: x.transpose(*d))((x @ wq).reshape(B, Sq, Hq, Dh), 0, 2, 1, 3)
        k = jnp.repeat(k_cache, rep, axis=1)
        v = jnp.repeat(v_cache, rep, axis=1)
        scores = jnp.einsum("bhqd,bhkd->bhqk", q, k) * (Dh ** -0.5)
        p = _softmax(scores, axis=-1)
        o = jnp.einsum("bhqk,bhkd->bhqd", p, v)
        return (lambda x, *d: x.transpose(*d))(o, 0, 2, 1, 3).reshape(B, Sq, Hq * Dh) @ wo

    def _B_ref(x, k_cache, v_cache, wq, wo):
        B, Sq, D = x.shape
        Hq, Dh = 32, 192
        Hkv = k_cache.shape[1]
        rep = Hq // Hkv
        q = (lambda x, *d: x.transpose(*d))((x @ wq).reshape(B, Sq, Hq, Dh), 0, 2, 1, 3)
        k = jnp.repeat(k_cache, rep, axis=1)
        v = jnp.repeat(v_cache, rep, axis=1)
        scores = jnp.einsum("bhqd,bhkd->bhqk", q, k) * (Dh ** -0.5)
        p = _softmax(scores, axis=-1)
        o = jnp.einsum("bhqk,bhkd->bhqd", p, v)
        return (lambda x, *d: x.transpose(*d))(o, 0, 2, 1, 3).reshape(B, Sq, Hq * Dh) @ wo

    a = _A_ref(A_x, A_k_cache, A_v_cache, A_wq, A_wo)
    b = _B_ref(B_x, B_k_cache, B_v_cache, B_wq, B_wo)
    return jnp.concatenate([a, b], axis=-1)
```

```python
import functools
import math

import jax
import jax.numpy as jnp
from jax import lax
import jax.experimental.pallas as pl
import jax.experimental.pallas.tpu as pltpu

NB, SQ, D = 8, 256, 640
H, SK, DH = 32, 1024, 192
PW = 2 * DH
NP = H // 2
NT = 2 * NB * NP
NBUF = 8
U = 2
QSCALE = (DH ** -0.5) * math.log2(math.e)
AH = NBUF - 1

def _kernel(ax, ak, av, awq, awo, bx, bk, bv, bwq, bwo, out,
            xbuf, kbuf, vbuf, wqbuf, wobuf, acc, obuf, qbuf, ohbuf, accA,
            ksem, vsem, xsem, wqsem, wosem, osem):

    def split(t):
        return (lax.shift_right_logical(t, 7), lax.shift_right_logical(t, 4) & 7, t & 15)

    def kv_copies(src_k, src_v, t):
        _, b, p = split(t)
        slot = t & (NBUF - 1)
        return (pltpu.make_async_copy(src_k.at[b, p], kbuf.at[slot], ksem.at[slot]),
                pltpu.make_async_copy(src_v.at[b, p], vbuf.at[slot], vsem.at[slot]))

    def w_copies(src_q, src_o, t):
        br, _, p = split(t)
        off = pl.multiple_of(p * PW, PW)
        return (pltpu.make_async_copy(src_q.at[:, pl.ds(off, PW)], wqbuf.at[br, p], wqsem.at[br, p]),
                pltpu.make_async_copy(src_o.at[pl.ds(off, PW), :], wobuf.at[br, p], wosem.at[br, p]))

    def x_copy(src_x, t):
        _, b, _ = split(t)
        slot = lax.shift_right_logical(t, 4) & 1
        return pltpu.make_async_copy(src_x.at[b], xbuf.at[slot], xsem.at[slot])

    def out_copy(t):
        br, b, _ = split(t)
        slot = lax.shift_right_logical(t, 4) & 1
        off = pl.multiple_of(br * D, D)
        return pltpu.make_async_copy(obuf.at[slot], out.at[b, :, pl.ds(off, D)], osem.at[slot])

    def start_step(t):
        br, b, p = split(t)

        def go(sx, sk, sv):
            for c in kv_copies(sk, sv, t):
                c.start()

            @pl.when(p == 0)
            def _():
                x_copy(sx, t).start()

        @pl.when(br == 0)
        def _():
            go(ax, ak, av)

            @pl.when(b == 0)
            def _():
                for c in w_copies(awq, awo, t):
                    c.start()

            @pl.when(b == 4)
            def _():
                for c in w_copies(bwq, bwo, t + 64):
                    c.start()

        @pl.when(br == 1)
        def _():
            go(bx, bk, bv)

    def wait_wx(t):
        br, b, p = split(t)

        @pl.when(b == 0)
        def _():
            for c in w_copies(awq, awo, t):
                c.wait()

        @pl.when(p == 0)
        def _():
            x_copy(ax, t).wait()

    lane = lax.broadcasted_iota(jnp.int32, (SQ, 128), 1)
    lo = lane < 64

    def qproj(t):
        br, b, p = split(t)
        xslot = lax.shift_right_logical(t, 4) & 1
        q = jnp.dot(xbuf[xslot], wqbuf[br, p], preferred_element_type=jnp.float32)
        q = (q * QSCALE).astype(jnp.bfloat16)
        q1 = q[:, 128:256]
        zero = jnp.zeros_like(q1)
        qbuf[0, :, 0:128] = q[:, 0:128]
        qbuf[0, :, 128:256] = jnp.where(lo, q1, zero)
        qbuf[1, :, 0:128] = jnp.where(lo, zero, q1)
        qbuf[1, :, 128:256] = q[:, 256:384]

    def oproj(t):
        br, b, p = split(t)
        return jnp.dot(ohbuf[...], wobuf[br, p], preferred_element_type=jnp.float32)

    start_step(jnp.int32(0))
    wait_wx(jnp.int32(0))
    for t0 in range(1, NBUF):
        start_step(jnp.int32(t0))
    qproj(jnp.int32(0))
    ohbuf[...] = jnp.zeros_like(ohbuf)
    acc[...] = jnp.zeros_like(acc)

    def attention(t, first, second, p0):
        slot = t & (NBUF - 1)
        tm = jnp.maximum(t - 1, 0)
        tn = jnp.minimum(t + 1, NT - 1)
        r = oproj(tm)
        if first:
            accA[...] = acc[...] + r
        elif second:
            acc[...] = jnp.where(p0, 0.0, accA[...]) + r
        else:
            acc[...] += r

        s0 = jnp.dot(qbuf[0], kbuf[slot, 0:256, :], preferred_element_type=jnp.float32)
        s1 = jnp.dot(qbuf[1], kbuf[slot, 128:384, :], preferred_element_type=jnp.float32)
        invs = []
        ots = []
        for hh, s in enumerate((s0, s1)):
            m = jnp.max(s, axis=1, keepdims=True)
            e = jnp.exp2(s - m)
            l = jnp.sum(e, axis=1, keepdims=True)
            invs.append(1.0 / l)
            vt = vbuf[slot, hh * DH:(hh + 1) * DH, :]
            ot = lax.dot_general(vt, e.astype(jnp.bfloat16), (((1,), (1,)), ((), ())),
                                 preferred_element_type=jnp.float32)
            ots.append(ot)
        qproj(tn)
        ot = jnp.concatenate(ots, axis=0)
        o = ot.T
        i0 = jnp.broadcast_to(invs[0], (SQ, 128))
        i1 = jnp.broadcast_to(invs[1], (SQ, 128))
        sc = jnp.concatenate([i0, jnp.where(lo, i0, i1), i1], axis=1)
        ohbuf[...] = (o * sc).astype(jnp.bfloat16)

    def body(i, carry):
        t = i * U
        p0 = (t & 15) == 0
        for u in range(U):
            for c in kv_copies(ak, av, t + u):
                c.wait()

        @pl.when(t + 1 < NT)
        def _():
            br, b, _ = split(t)
            @pl.when(b == 0)
            def _():
                for u in range(1, U):
                    for c in w_copies(awq, awo, t + u):
                        c.wait()
            @pl.when(t + U < NT)
            def _():
                wait_wx(t + U)

        for u in range(U):
            attention(t + u, u == 0, u == 1, p0)

        @pl.when(t + NBUF < NT)
        def _():
            for u in range(U):
                start_step(t + NBUF + u)

        @pl.when(p0 & (t > 0))
        def _():
            tm = t - 1
            xs = lax.shift_right_logical(tm, 4) & 1
            @pl.when(t > 2 * NP)
            def _():
                out_copy(tm - 2 * NP).wait()
            obuf[xs] = accA[...].astype(jnp.bfloat16)
            out_copy(tm).start()

        return carry

    lax.fori_loop(0, NT // U, body, 0)
    tl = jnp.int32(NT - 1)
    r = acc[...] + oproj(tl)
    out_copy(jnp.int32(NT - 1 - 2 * NP)).wait()
    obuf[1] = r.astype(jnp.bfloat16)
    out_copy(tl).start()
    out_copy(jnp.int32(NT - 1 - NP)).wait()
    out_copy(tl).wait()


@jax.jit
def pallas_concat_heads__gqa_block_cached__gqa_block_cached__near_ridge_kernel(
    A_x, A_k_cache, A_v_cache, A_wq, A_wo, B_x, B_k_cache, B_v_cache, B_wq, B_wo,
):
    def tr(c):
        return jnp.swapaxes(c, 2, 3).reshape(NB, NP, PW, SK)

    any_spec = pl.BlockSpec(memory_space=pl.ANY)
    return pl.pallas_call(
        _kernel,
        in_specs=[any_spec] * 10,
        out_specs=any_spec,
        out_shape=jax.ShapeDtypeStruct((NB, SQ, 2 * D), jnp.bfloat16),
        scratch_shapes=[
            pltpu.VMEM((2, SQ, D), jnp.bfloat16),
            pltpu.VMEM((NBUF, PW, SK), jnp.bfloat16),
            pltpu.VMEM((NBUF, PW, SK), jnp.bfloat16),
            pltpu.VMEM((2, NP, D, PW), jnp.bfloat16),
            pltpu.VMEM((2, NP, PW, D), jnp.bfloat16),
            pltpu.VMEM((SQ, D), jnp.float32),
            pltpu.VMEM((2, SQ, D), jnp.bfloat16),
            pltpu.VMEM((2, SQ, 256), jnp.bfloat16),
            pltpu.VMEM((SQ, PW), jnp.bfloat16),
            pltpu.VMEM((SQ, D), jnp.float32),
            pltpu.SemaphoreType.DMA((NBUF,)),
            pltpu.SemaphoreType.DMA((NBUF,)),
            pltpu.SemaphoreType.DMA((2,)),
            pltpu.SemaphoreType.DMA((2, NP)),
            pltpu.SemaphoreType.DMA((2, NP)),
            pltpu.SemaphoreType.DMA((2,)),
        ],
        compiler_params=pltpu.CompilerParams(vmem_limit_bytes=100 * 1024 * 1024),
    )(A_x, tr(A_k_cache), tr(A_v_cache), A_wq, A_wo,
      B_x, tr(B_k_cache), tr(B_v_cache), B_wq, B_wo)
```

```python
import functools
import math

import jax
import jax.numpy as jnp
from jax import lax
import jax.experimental.pallas as pl
import jax.experimental.pallas.tpu as pltpu

NB, SQ, D = 8, 256, 640
H, SK, DH = 32, 1024, 192
PW = 2 * DH
NP = H // 2
NT = 2 * NB * NP
NBUF = 8
U = 2
QSCALE = (DH ** -0.5) * math.log2(math.e)
AH = NBUF - 1

def _kernel(ax, ak, av, awq, awo, bx, bk, bv, bwq, bwo, out,
            xbuf, kbuf, vbuf, wqbuf, wobuf, acc, obuf, qbuf, ohbuf, accA,
            ksem, vsem, xsem, wqsem, wosem, osem):

    def split(t):
        return (lax.shift_right_logical(t, 7), lax.shift_right_logical(t, 4) & 7, t & 15)

    def kv_copies(src_k, src_v, t):
        _, b, p = split(t)
        slot = t & (NBUF - 1)
        return (pltpu.make_async_copy(src_k.at[b, p], kbuf.at[slot], ksem.at[slot]),
                pltpu.make_async_copy(src_v.at[b, p], vbuf.at[slot], vsem.at[slot]))

    def w_copies(src_q, src_o, t):
        br, _, p = split(t)
        off = pl.multiple_of(p * PW, PW)
        return (pltpu.make_async_copy(src_q.at[:, pl.ds(off, PW)], wqbuf.at[br, p], wqsem.at[br, p]),
                pltpu.make_async_copy(src_o.at[pl.ds(off, PW), :], wobuf.at[br, p], wosem.at[br, p]))

    def x_copy(src_x, t):
        _, b, _ = split(t)
        slot = lax.shift_right_logical(t, 4) & 1
        return pltpu.make_async_copy(src_x.at[b], xbuf.at[slot], xsem.at[slot])

    def out_copy(t):
        br, b, _ = split(t)
        slot = lax.shift_right_logical(t, 4) & 1
        off = pl.multiple_of(br * D, D)
        return pltpu.make_async_copy(obuf.at[slot], out.at[b, :, pl.ds(off, D)], osem.at[slot])

    def start_step(t):
        br, b, p = split(t)

        def go(sx, sk, sv):
            for c in kv_copies(sk, sv, t):
                c.start()

            @pl.when(p == 0)
            def _():
                x_copy(sx, t).start()

        @pl.when(br == 0)
        def _():
            go(ax, ak, av)

            @pl.when(b == 0)
            def _():
                for c in w_copies(awq, awo, t):
                    c.start()

            @pl.when(b == 4)
            def _():
                for c in w_copies(bwq, bwo, t + 64):
                    c.start()

        @pl.when(br == 1)
        def _():
            go(bx, bk, bv)

    def wait_wx(t):
        br, b, p = split(t)

        @pl.when(b == 0)
        def _():
            for c in w_copies(awq, awo, t):
                c.wait()

        @pl.when(p == 0)
        def _():
            x_copy(ax, t).wait()

    lane = lax.broadcasted_iota(jnp.int32, (SQ, 128), 1)
    lo = lane < 64

    def qproj(t):
        br, b, p = split(t)
        xslot = lax.shift_right_logical(t, 4) & 1
        q = jnp.dot(xbuf[xslot], wqbuf[br, p], preferred_element_type=jnp.float32)
        q = (q * QSCALE).astype(jnp.bfloat16)
        q1 = q[:, 128:256]
        zero = jnp.zeros_like(q1)
        qbuf[0, :, 0:128] = q[:, 0:128]
        qbuf[0, :, 128:256] = jnp.where(lo, q1, zero)
        qbuf[1, :, 0:128] = jnp.where(lo, zero, q1)
        qbuf[1, :, 128:256] = q[:, 256:384]

    def oproj(t):
        br, b, p = split(t)
        return jnp.dot(ohbuf[...], wobuf[br, p], preferred_element_type=jnp.float32)

    start_step(jnp.int32(0))
    wait_wx(jnp.int32(0))
    for t0 in range(1, NBUF):
        start_step(jnp.int32(t0))
    qproj(jnp.int32(0))
    ohbuf[...] = jnp.zeros_like(ohbuf)
    acc[...] = jnp.zeros_like(acc)

    def attention(t, first, second, p0):
        slot = t & (NBUF - 1)
        tm = jnp.maximum(t - 1, 0)
        tn = jnp.minimum(t + 1, NT - 1)
        s0 = jnp.dot(qbuf[0], kbuf[slot, 0:256, :], preferred_element_type=jnp.float32)
        r = oproj(tm)
        if first:
            a0 = acc[...] + r
            accA[...] = a0
            obuf[lax.shift_right_logical(tm, 4) & 1] = a0.astype(jnp.bfloat16)
        elif second:
            acc[...] = jnp.where(p0, 0.0, accA[...]) + r
        else:
            acc[...] += r

        s1 = jnp.dot(qbuf[1], kbuf[slot, 128:384, :], preferred_element_type=jnp.float32)
        invs = []
        ots = []
        for hh, s in enumerate((s0, s1)):
            m = jnp.max(s, axis=1, keepdims=True)
            e = jnp.exp2(s - m)
            l = jnp.sum(e, axis=1, keepdims=True)
            invs.append(1.0 / l)
            vt = vbuf[slot, hh * DH:(hh + 1) * DH, :]
            ot = lax.dot_general(vt, e.astype(jnp.bfloat16), (((1,), (1,)), ((), ())),
                                 preferred_element_type=jnp.float32)
            ots.append(ot)
        qproj(tn)

        @pl.when(t + NBUF < NT)
        def _():
            start_step(t + NBUF)

        ot = jnp.concatenate(ots, axis=0)
        o = ot.T
        i0 = jnp.broadcast_to(invs[0], (SQ, 128))
        i1 = jnp.broadcast_to(invs[1], (SQ, 128))
        sc = jnp.concatenate([i0, jnp.where(lo, i0, i1), i1], axis=1)
        ohbuf[...] = (o * sc).astype(jnp.bfloat16)

    def body(i, carry):
        t = i * U
        p0 = (t & 15) == 0
        for u in range(U):
            for c in kv_copies(ak, av, t + u):
                c.wait()

        @pl.when(t + 1 < NT)
        def _():
            br, b, _ = split(t)
            @pl.when(b == 0)
            def _():
                for u in range(1, U):
                    for c in w_copies(awq, awo, t + u):
                        c.wait()
            @pl.when(t + U < NT)
            def _():
                wait_wx(t + U)

        for u in range(U):
            attention(t + u, u == 0, u == 1, p0)

        @pl.when(p0 & (t > 0))
        def _():
            out_copy(t - 1).start()

            @pl.when(t > NP)
            def _():
                out_copy(t - 1 - NP).wait()

        return carry

    lax.fori_loop(0, NT // U, body, 0)
    tl = jnp.int32(NT - 1)
    r = acc[...] + oproj(tl)
    obuf[1] = r.astype(jnp.bfloat16)
    out_copy(tl).start()
    out_copy(jnp.int32(NT - 1 - NP)).wait()
    out_copy(tl).wait()


@jax.jit
def pallas_concat_heads__gqa_block_cached__gqa_block_cached__near_ridge_kernel(
    A_x, A_k_cache, A_v_cache, A_wq, A_wo, B_x, B_k_cache, B_v_cache, B_wq, B_wo,
):
    def tr(c):
        return jnp.swapaxes(c, 2, 3).reshape(NB, NP, PW, SK)

    any_spec = pl.BlockSpec(memory_space=pl.ANY)
    return pl.pallas_call(
        _kernel,
        in_specs=[any_spec] * 10,
        out_specs=any_spec,
        out_shape=jax.ShapeDtypeStruct((NB, SQ, 2 * D), jnp.bfloat16),
        scratch_shapes=[
            pltpu.VMEM((2, SQ, D), jnp.bfloat16),
            pltpu.VMEM((NBUF, PW, SK), jnp.bfloat16),
            pltpu.VMEM((NBUF, PW, SK), jnp.bfloat16),
            pltpu.VMEM((2, NP, D, PW), jnp.bfloat16),
            pltpu.VMEM((2, NP, PW, D), jnp.bfloat16),
            pltpu.VMEM((SQ, D), jnp.float32),
            pltpu.VMEM((2, SQ, D), jnp.bfloat16),
            pltpu.VMEM((2, SQ, 256), jnp.bfloat16),
            pltpu.VMEM((SQ, PW), jnp.bfloat16),
            pltpu.VMEM((SQ, D), jnp.float32),
            pltpu.SemaphoreType.DMA((NBUF,)),
            pltpu.SemaphoreType.DMA((NBUF,)),
            pltpu.SemaphoreType.DMA((2,)),
            pltpu.SemaphoreType.DMA((2, NP)),
            pltpu.SemaphoreType.DMA((2, NP)),
            pltpu.SemaphoreType.DMA((2,)),
        ],
        compiler_params=pltpu.CompilerParams(vmem_limit_bytes=100 * 1024 * 1024, flags={'XLA_TPU_MAX_INSTS_TO_PREDICATE': 65536}),
    )(A_x, tr(A_k_cache), tr(A_v_cache), A_wq, A_wo,
      B_x, tr(B_k_cache), tr(B_v_cache), B_wq, B_wo)
```
